```python
import os as _os
_os.environ.setdefault("JAX_PLATFORMS", "cpu")
import jax
import jax.numpy as jnp

def _softmax(x, axis=-1):
    return jax.nn.softmax(x, axis=axis)
def _gelu(x):
    return jax.nn.gelu(x, approximate=True)
def _silu(x):
    return jax.nn.silu(x)
def _sigmoid(x):
    return jax.nn.sigmoid(x)
def _layernorm(x, axis=-1, eps=1e-5):
    m = jnp.mean(x, axis=axis, keepdims=True)
    v = jnp.var(x, axis=axis, keepdims=True)
    return (x - m) / jnp.sqrt(v + eps)
def _scatter_add(tgt, idx, src, axis=0):
    return tgt.at[idx].add(src)
def _segment_sum(src, seg, n):
    return jax.ops.segment_sum(src, seg, n)
class _Rng:
    def __init__(self, key):
        self._k = key
    def _next(self):
        self._k, sub = jax.random.split(self._k)
        return sub
    def normal(self, shape):
        return jax.random.normal(self._next(), shape, dtype=jnp.bfloat16)
    def randint(self, lo, hi, shape):
        return jax.random.randint(self._next(), shape, lo, hi, dtype=jnp.int32)
    def uniform(self, shape, lo=0.0, hi=1.0):
        return jax.random.uniform(self._next(), shape, jnp.bfloat16, lo, hi)
    def permutation(self, n):
        return jax.random.permutation(self._next(), n)


kernel_name = 'interleave_layers__sliding_local_dilated__mixer_channel_mlp__prompt'

def setup_inputs():
    _rng = _Rng(jax.random.key(int.from_bytes(__import__("os").urandom(4), "little")))
    _w = (lambda a: (lambda t: t.astype(jnp.bfloat16) if jnp.issubdtype(t.dtype, jnp.floating) else t)(jnp.asarray(a)))
    def _A_setup():
        B, S, D = 1, 2048, 512
        return {
            "x": _w((lambda *s: _rng.normal(s) * 0.05)(B, S, D)),
            "wqkv": _w((lambda *s: _rng.normal(s) * 0.05)(D, 3 * D)),
            "wo": _w((lambda *s: _rng.normal(s) * 0.05)(D, D)),
        }
    _A_in = _A_setup()

    def _B_setup():
        B, S, D, F = 1, 2048, 512, 1376
        return {
            "x": _w((lambda *s: _rng.normal(s) * 0.05)(B, S, D)),
            "w1": _w((lambda *s: _rng.normal(s) * 0.4)(D, F) * (D ** -0.5)),
            "b1": _w((lambda *s: _rng.normal(s) * 0.4)(F)),
            "w2": _w((lambda *s: _rng.normal(s) * 0.4)(F, D) * (F ** -0.5)),
            "b2": _w((lambda *s: _rng.normal(s) * 0.4)(D)),
        }
    _B_in = _B_setup()

    return {
        "A_x": _A_in["x"],
        "A_wqkv": _A_in["wqkv"],
        "A_wo": _A_in["wo"],
        "B_x": _B_in["x"],
        "B_w1": _B_in["w1"],
        "B_b1": _B_in["b1"],
        "B_w2": _B_in["w2"],
        "B_b2": _B_in["b2"],
    }

def reference(A_x, A_wqkv, A_wo, B_x, B_w1, B_b1, B_w2, B_b2):
    def _A_ref(x, wqkv, wo):
        B, S, D = x.shape
        H = 32; Dh = D // H
        W, dil = 8, 2
        qkv = (lambda x, *d: x.transpose(*d))((x @ wqkv).reshape(B, S, 3, H, Dh), 2, 0, 3, 1, 4)
        q, k, v = qkv[0], qkv[1], qkv[2]
        scale = Dh ** -0.5
        pos = jnp.arange(S)
        off = jnp.arange(W) * dil
        idx = pos[:, None] - off[None, :]
        mask = idx >= 0
        idx_c = jnp.where(mask, idx, 0).reshape(-1)
        kg = k[:, :, idx_c, :].reshape(B, H, S, W, Dh)
        vg = v[:, :, idx_c, :].reshape(B, H, S, W, Dh)
        logits = jnp.einsum("bhsd,bhswd->bhsw", q, kg) * scale
        logits = jnp.where(mask[None, None, :, :], logits, -1e9)
        attn = _softmax(logits, axis=-1)
        o = jnp.einsum("bhsw,bhswd->bhsd", attn, vg)
        return (lambda x, *d: x.transpose(*d))(o, 0, 2, 1, 3).reshape(B, S, D) @ wo

    def _B_ref(x, w1, b1, w2, b2):
        y = _layernorm(x, axis=-1)
        h = _gelu(jnp.einsum("bsd,df->bsf", y, w1) + b1)
        return jnp.einsum("bsf,fd->bsd", h, w2) + b2

    x = A_x
    x = x + _A_ref(_layernorm(x, axis=-1), A_wqkv, A_wo)
    x = x + _B_ref(_layernorm(x, axis=-1), B_w1, B_b1, B_w2, B_b2)
    x = x + _A_ref(_layernorm(x, axis=-1), A_wqkv, A_wo)
    x = x + _B_ref(_layernorm(x, axis=-1), B_w1, B_b1, B_w2, B_b2)
    return x
```

```python
import functools
import os
import jax
import jax.numpy as jnp
import jax.experimental.pallas as pl
import jax.experimental.pallas.tpu as pltpu

S, D, F = 2048, 512, 1376
H, DH, W, DIL = 32, 16, 8, 2
EPS = 1e-5
HALO = 16
SUB = int(os.environ.get('SUB', 128))
TM = 2 * SUB
NIT = S // TM
LA = 2
RB = int(os.environ.get('RB', 16))
CK = int(os.environ.get('CK', 0))
NQ = max(CK, 1)
LB = int(os.environ.get('LB', 32))
WCH = 4
bf16, f32, u32, i32 = jnp.bfloat16, jnp.float32, jnp.uint32, jnp.int32


def _stats(x):
    m = jnp.sum(x, axis=-1, keepdims=True) * (1.0 / D)
    xc = x - m
    v = jnp.sum(xc * xc, axis=-1, keepdims=True) * (1.0 / D)
    return xc, v


def _ln(x):
    xc, v = _stats(x)
    return xc * jax.lax.rsqrt(v + EPS)


def _ln_ln(x):
    xc, v = _stats(x)
    return xc * jax.lax.rsqrt(v * (1.0 + EPS) + EPS * EPS)


def _gelu(h):
    c = 0.7978845608028654
    u = h * (c + (c * 0.044715) * (h * h))
    hh = 0.5 * h
    return hh + hh * jnp.tanh(u)


def _tree(op, xs):
    xs = list(xs)
    while len(xs) > 1:
        nxt = [op(xs[k], xs[k + 1]) for k in range(0, len(xs) - 1, 2)]
        if len(xs) % 2:
            nxt.append(xs[-1])
        xs = nxt
    return xs[0]


def _recip(d):
    r = pl.reciprocal(d, approx=True)
    return r * (2.0 - d * r)


def _pk(v):
    return pltpu.bitcast(v.astype(bf16), u32)


def _up(v):
    return pltpu.bitcast(v, bf16)


def _sel4(sel, vals):
    return jnp.where(sel < 2, jnp.where(sel == 0, vals[0], vals[1]),
                     jnp.where(sel == 2, vals[2], vals[3]))


def _kernel(x_hbm, wqkv_hbm, wo_hbm, w1t_hbm, b1_hbm, w2_hbm, b2_hbm, o_hbm,
            x_v, o_v, wqkv_v, wo_v, w1t_v, w2_v, b1_v, b2_v,
            wqkv_p, wo_p, b1_s, b2_s, kv_s, z_s, sem, osem, *bufs):
    x_s = bufs[0:2]
    g_s = bufs[2:4]
    x1_s = bufs[4:6]
    y2_s = bufs[6:8]
    y_s = bufs[8:12]
    q_bufs = bufs[12:]
    RW = D // WCH

    X0 = LA * TM
    cp_x0 = pltpu.make_async_copy(x_hbm.at[0:TM], x_v.at[0:TM], sem.at[0])
    cp_wq = [pltpu.make_async_copy(wqkv_hbm.at[r * RW:(r + 1) * RW], wqkv_v.at[r * RW:(r + 1) * RW],
                                   sem.at[1 + r]) for r in range(WCH)]
    cp_wo = pltpu.make_async_copy(wo_hbm, wo_v, sem.at[1 + WCH])
    cp_b1 = pltpu.make_async_copy(b1_hbm, b1_v, sem.at[2 + WCH])
    cp_b2 = pltpu.make_async_copy(b2_hbm, b2_v, sem.at[3 + WCH])
    cp_w1 = pltpu.make_async_copy(w1t_hbm, w1t_v, sem.at[4 + WCH])
    cp_w2 = pltpu.make_async_copy(w2_hbm, w2_v, sem.at[5 + WCH])
    cp_x1 = pltpu.make_async_copy(x_hbm.at[TM:X0], x_v.at[TM:X0], sem.at[6 + WCH])
    cp_x2 = pltpu.make_async_copy(x_hbm.at[X0:X0 + TM], x_v.at[X0:X0 + TM], sem.at[7 + WCH])
    cp_xr = pltpu.make_async_copy(x_hbm.at[X0 + TM:S], x_v.at[X0 + TM:S], sem.at[8 + WCH])

    def cp_out(row, n):
        return pltpu.make_async_copy(o_v.at[pl.ds(row, n)], o_hbm.at[pl.ds(row, n)], osem)

    cp_x0.start()
    for c in cp_wq:
        c.start()
    cp_wo.start()
    cp_x1.start()
    cp_b1.start()
    cp_b2.start()
    cp_w1.start()
    cp_w2.start()
    cp_x2.start()

    z_s[0] = 0
    kv_s[:, :, 0:HALO, :] = jnp.zeros((2, 8, HALO, 128), f32)
    zz = [0]

    def qslot(cid, rb):
        return q_bufs[cid * NQ + rb % NQ], (rb // NQ) * RB

    def load_q(cid, rb, c):
        buf, r = qslot(cid, rb)
        if CK:
            return buf[c, pl.ds(zz[0] + r, RB), :]
        return buf[c, r:r + RB, :]

    def attn_block(j, layer, rb, row0):
        cid = 2 * layer + j
        base = j * SUB
        r0 = rb * RB
        q = [load_q(cid, rb, c) for c in range(4)]
        lg = []
        for w in range(W):
            st = HALO + base + r0 - DIL * w
            s = _tree(jnp.add, [q[c] * kv_s[layer, c, st:st + RB, :] for c in range(4)])
            s = s + pltpu.roll(s, 64, 1)
            s = s + pltpu.roll(s, 32, 1)
            if j == 0 and r0 < DIL * w and not (isinstance(row0, int) and row0 > 0):
                pos = row0 + r0 + jax.lax.broadcasted_iota(i32, (RB, 128), 0)
                s = jnp.where(pos >= DIL * w, s, -1e9)
            lg.append(s)
        m = _tree(jnp.maximum, lg)
        e = [jnp.exp(l - m) for l in lg]
        inv = _recip(_tree(jnp.add, e))
        for c in range(4):
            st = HALO + base + r0
            acc = _tree(jnp.add, [e[w] * kv_s[layer, 4 + c, st - DIL * w:st - DIL * w + RB, :]
                                  for w in range(W)])
            acc = acc * inv
            y_s[cid][r0 // 2:(r0 + RB) // 2, c * 128:(c + 1) * 128] = _pk(acc)
        if CK:
            buf, _ = qslot(cid, rb)
            buf[4, 0:8, :] = acc[0:8]

    def ln_stage(fn, load, store):
        for lb in range(SUB // LB):
            r0 = lb * LB
            store(r0 // 2, LB // 2, _pk(fn(load(r0, LB))))

    def set_rows(ref, *lead):
        def store(r, n, v):
            ref[(*lead, slice(r, r + n), slice(None))] = v
        return store

    def get_rows(ref, *lead):
        return lambda r, n: ref[(*lead, slice(r, r + n), slice(None))]

    def ln_in(j, row0):
        ln_stage(_ln, lambda r, n: x_v[pl.ds(row0 + r, n), :].astype(f32), set_rows(y_s[j]))

    def st_q(j, layer):
        cid = 2 * layer + j
        base = j * SUB
        qkv = jnp.dot(_up(y_s[cid][...]), _up(wqkv_p[...]), preferred_element_type=f32)
        for c in range(12):
            blk = qkv[:, c * 128:(c + 1) * 128]
            if c < 4:
                for rb in range(SUB // RB):
                    buf, r = qslot(cid, rb)
                    buf[c, r:r + RB, :] = blk[rb * RB:(rb + 1) * RB]
            else:
                kv_s[layer, c - 4, HALO + base:HALO + base + SUB, :] = blk

    def st_o(j, layer, row0, slot=None):
        cid = 2 * layer + j
        for rb in range(SUB // RB):
            attn_block(j, layer, rb, row0)
        if j == 1:
            kv_s[layer, :, 0:HALO, :] = kv_s[layer, :, TM:TM + HALO, :]
        att = jnp.dot(_up(y_s[cid][...]), _up(wo_p[...]), preferred_element_type=f32)
        if layer == 0:
            x1_s[j][slot] = x_v[pl.ds(row0, SUB), :].astype(f32) + att
            ln_stage(_ln_ln, get_rows(x1_s[j], slot), set_rows(y2_s[j], slot))
        else:
            x_s[j][...] = x_s[j][...] + att
            ln_stage(_ln_ln, get_rows(x_s[j]), set_rows(y_s[cid]))

    def st_u(j, layer, slot=None):
        y = y2_s[j][slot] if layer == 0 else y_s[2 + j][...]
        h = jax.lax.dot_general(_up(y), w1t_v[...], (((1,), (1,)), ((), ())),
                                preferred_element_type=f32) + b1_s[...]
        g_s[j][...] = _pk(_gelu(h))

    def st_d(j, layer, row0, slot=None):
        mlp = jnp.dot(_up(g_s[j][...]), w2_v[...], preferred_element_type=f32) + b2_s[...]
        if layer == 0:
            x_s[j][...] = x1_s[j][slot] + mlp
            ln_stage(_ln, get_rows(x_s[j]), set_rows(y_s[2 + j]))
        else:
            o_v[pl.ds(row0, SUB), :] = (x_s[j][...] + mlp).astype(bf16)

    cp_x0.wait()
    ln_in(0, 0)
    ln_in(1, SUB)
    lam = jax.lax.broadcasted_iota(i32, (128, 128), 0)
    n = jax.lax.broadcasted_iota(i32, (128, 128), 1)

    def perm(a, b, j):
        return (b == (a % 4) * 32 + (((a // 4) % 4 - j) % 4) * 8 + a // 16).astype(bf16)

    p = [perm(lam, n, j) for j in range(4)]
    pt = [perm(n, lam, j) for j in range(4)]
    dhi_l = (jax.lax.broadcasted_iota(i32, (RW // 2, 128), 1) // 4) % 4
    for r in range(WCH):
        cp_wq[r].wait()
        for t in range(3):
            src = [pltpu.bitcast(wqkv_v[r * RW:(r + 1) * RW, t * D + c * 128:t * D + (c + 1) * 128], u32)
                   for c in range(4)]
            for j in range(4):
                mixed = _sel4((dhi_l - j) % 4, src)
                res = jnp.dot(_up(mixed), p[j], preferred_element_type=f32)
                if t == 0:
                    res = res * (DH ** -0.5)
                wqkv_p[r * RW // 2:(r + 1) * RW // 2, t * D + j * 128:t * D + (j + 1) * 128] = _pk(res)
    st_q(0, 0)
    cp_wo.wait()
    cp_x1.wait()
    dhi_r = (jax.lax.broadcasted_iota(i32, (64, D), 0) // 2) % 4
    src = [pltpu.bitcast(wo_v[c * 128:(c + 1) * 128, :], u32) for c in range(4)]
    for j in range(4):
        mixed = _sel4((dhi_r - j) % 4, src)
        wo_p[j * 64:(j + 1) * 64, :] = _pk(jnp.dot(pt[j], _up(mixed), preferred_element_type=f32))
    st_q(1, 0)
    st_o(0, 0, 0, 0)
    for a in range(1, LA):
        ln_in(0, a * TM)
        st_o(1, 0, (a - 1) * TM + SUB, a - 1)
        st_q(0, 0)
        ln_in(1, a * TM + SUB)
        st_q(1, 0)
        st_o(0, 0, a * TM, a)
    st_o(1, 0, (LA - 1) * TM + SUB, LA - 1)
    cp_b1.wait()
    cp_b2.wait()
    b1_s[...] = b1_v[...].astype(f32).reshape(1, F)
    b2_s[...] = b2_v[...].astype(f32).reshape(1, D)
    cp_w1.wait()
    cp_w2.wait()
    cp_x2.wait()
    cp_xr.start()

    def steady(k, ahead):
        rx = pl.multiple_of(k * TM, TM)
        ry = pl.multiple_of(rx + SUB, SUB)
        rn = pl.multiple_of(rx + LA * TM, TM)
        rm = pl.multiple_of(rn + SUB, SUB)
        slot = k % LA
        zz[0] = k >> 16
        st_u(0, 0, slot)
        if ahead:
            ln_in(0, rn)
            st_q(0, 0)
        st_d(0, 0, rx, slot)
        st_u(1, 0, slot)
        if ahead:
            st_o(0, 0, rn, slot)
        st_q(0, 1)
        st_d(1, 0, ry, slot)
        st_o(0, 1, rx)
        st_q(1, 1)
        st_u(0, 1)
        st_o(1, 1, ry)
        if ahead:
            ln_in(1, rm)
            st_q(1, 0)
        st_d(0, 1, rx)
        st_u(1, 1)
        if ahead:
            st_o(1, 0, rm, slot)
        st_d(1, 1, ry)
        cp_out(rx, TM).start()

    def body1(k, carry):
        @pl.when(k == 1)
        def _():
            cp_xr.wait()
        steady(k, True)
        return carry

    def body2(k, carry):
        steady(k, False)
        return carry

    jax.lax.fori_loop(0, NIT - LA, body1, 0)
    jax.lax.fori_loop(NIT - LA, NIT, body2, 0)
    for t in range(NIT):
        cp_out(t * TM, TM).wait()


@jax.jit
def pallas_interleave_layers__sliding_local_dilated__mixer_channel_mlp__prompt_kernel(
    A_x, A_wqkv, A_wo, B_x, B_w1, B_b1, B_w2, B_b2):
    x = A_x.reshape(S, D)
    nblk = SUB // RB
    qrows = -(-nblk // NQ) * RB
    anyspec = pl.BlockSpec(memory_space=pl.ANY)
    out = pl.pallas_call(
        _kernel,
        in_specs=[anyspec] * 7,
        out_specs=anyspec,
        out_shape=jax.ShapeDtypeStruct((S, D), bf16),
        scratch_shapes=[
            pltpu.VMEM((S, D), bf16),
            pltpu.VMEM((S, D), bf16),
            pltpu.VMEM((D, 3 * D), bf16),
            pltpu.VMEM((D, D), bf16),
            pltpu.VMEM((F, D), bf16),
            pltpu.VMEM((F, D), bf16),
            pltpu.VMEM((F,), bf16),
            pltpu.VMEM((D,), bf16),
            pltpu.VMEM((D // 2, 3 * D), u32),
            pltpu.VMEM((D // 2, D), u32),
            pltpu.VMEM((1, F), f32),
            pltpu.VMEM((1, D), f32),
            pltpu.VMEM((2, 8, TM + HALO, 128), f32),
            pltpu.SMEM((1,), i32),
            pltpu.SemaphoreType.DMA((9 + WCH,)),
            pltpu.SemaphoreType.DMA,
        ] + [pltpu.VMEM((SUB, D), f32) for _ in range(2)]
          + [pltpu.VMEM((SUB // 2, F), u32) for _ in range(2)]
          + [pltpu.VMEM((LA, SUB, D), f32) for _ in range(2)]
          + [pltpu.VMEM((LA, SUB // 2, D), u32) for _ in range(2)]
          + [pltpu.VMEM((SUB // 2, D), u32) for _ in range(4)]
          + [pltpu.VMEM((5, qrows, 128), f32) for _ in range(NQ * 4)],
        compiler_params=pltpu.CompilerParams(
            vmem_limit_bytes=100 * 1024 * 1024,
        ),
    )(x, A_wqkv, A_wo, B_w1.T, B_b1, B_w2, B_b2)
    return out.reshape(1, S, D)
```

```python
import functools
import math

import jax
import jax.numpy as jnp
import jax.experimental.pallas as pl
import jax.experimental.pallas.tpu as pltpu

S, D, F = 2048, 512, 1376
H, DH, W, DIL = 32, 16, 8, 2
EPS = 1e-5
SCALE = DH ** -0.5
HALO = 16
KPAD = 8
SUB = 128
TM = 2 * SUB
NIT = S // TM
LA = 2
RB = 16
LB = 32
PR = 64
bf16, f32, u32, i32 = jnp.bfloat16, jnp.float32, jnp.uint32, jnp.int32


def _stats(x):
    m = jnp.sum(x, axis=-1, keepdims=True) * (1.0 / D)
    xc = x - m
    v = jnp.sum(xc * xc, axis=-1, keepdims=True) * (1.0 / D)
    return xc, v


def _ln(x):
    xc, v = _stats(x)
    return xc * jax.lax.rsqrt(v + EPS)


def _ln_ln(x):
    xc, v = _stats(x)
    return xc * jax.lax.rsqrt(v * (1.0 + EPS) + EPS * EPS)


def _gelu(h):
    c = math.sqrt(2.0 / math.pi)
    u = h * (c + (c * 0.044715) * (h * h))
    hh = 0.5 * h
    return hh + hh * jnp.tanh(u)


def _tree(op, xs):
    xs = list(xs)
    while len(xs) > 1:
        nxt = [op(xs[k], xs[k + 1]) for k in range(0, len(xs) - 1, 2)]
        if len(xs) % 2:
            nxt.append(xs[-1])
        xs = nxt
    return xs[0]


def _recip(d):
    r = pl.reciprocal(d, approx=True)
    return r * (2.0 - d * r)


def _pk(v):
    return pltpu.bitcast(v.astype(bf16), u32)


def _up(v):
    return pltpu.bitcast(v, bf16)


def _sel4(sel, vals):
    return jnp.where(sel < 2, jnp.where(sel == 0, vals[0], vals[1]),
                     jnp.where(sel == 2, vals[2], vals[3]))


def _kernel(x_hbm, wqkv_hbm, wo_hbm, w1t_hbm, b1_hbm, w2_hbm, b2_hbm, o_hbm,
            x_v, o_v, wqkv_v, wo_v, w1t_v, w2_v, b1_v, b2_v,
            wqkv_p, wo_p, pt_s, zero_s, b1_s, b2_s, kv0_s, kv1_s, sem, osem, *bufs):
    x_s = bufs[0:2]
    g_s = bufs[2:4]
    x1_s = bufs[4:6]
    y2_s = bufs[6:8]
    y_s = bufs[8:12]
    q_s = bufs[12:16]

    def cp_x(lo, hi, s):
        return pltpu.make_async_copy(x_hbm.at[lo:hi], x_v.at[lo:hi], sem.at[s])

    cps = {
        'x0': cp_x(0, TM, 0),
        'Wq': pltpu.make_async_copy(wqkv_hbm.at[:, 0:D], wqkv_v.at[0], sem.at[1]),
        'Wk': pltpu.make_async_copy(wqkv_hbm.at[:, D:2 * D], wqkv_v.at[1], sem.at[2]),
        'Wv': pltpu.make_async_copy(wqkv_hbm.at[:, 2 * D:3 * D], wqkv_v.at[2], sem.at[3]),
        'wo': pltpu.make_async_copy(wo_hbm, wo_v, sem.at[4]),
        'x1': cp_x(TM, LA * TM, 5),
        'b1': pltpu.make_async_copy(b1_hbm, b1_v, sem.at[6]),
        'b2': pltpu.make_async_copy(b2_hbm, b2_v, sem.at[7]),
        'w1': pltpu.make_async_copy(w1t_hbm, w1t_v, sem.at[8]),
        'w2': pltpu.make_async_copy(w2_hbm, w2_v, sem.at[9]),
        'x2': cp_x(LA * TM, (LA + 1) * TM, 10),
    }
    cp_xr = cp_x((LA + 1) * TM, S, 11)

    def cp_out(row):
        return pltpu.make_async_copy(o_v.at[pl.ds(row, SUB)], o_hbm.at[pl.ds(row, SUB)], osem)

    for cp in cps.values():
        cp.start()

    kv0_s[:, 0:HALO, :] = jnp.zeros((8, HALO, 128), f32)
    kv1_s[:, 0:HALO, :] = jnp.zeros((8, HALO, 128), f32)
    zero_s[...] = jnp.zeros(zero_s.shape, i32)

    src_id = jax.lax.broadcasted_iota(i32, (128, 128), 1)
    dst_id = jax.lax.broadcasted_iota(i32, (128, 128), 0)
    for j in range(4):
        hit = dst_id == (src_id % 4) * 32 + (((src_id // 4) % 4 - j) % 4) * 8 + src_id // 16
        pt_s[j] = _pk(jnp.where(hit, 1.0, 0.0))

    def attn_block(ctx, rb, row0, tok):
        b, kv, base = ctx
        r0 = rb * RB
        last = rb == SUB // RB - 1
        q = [q_s[b][c, r0:r0 + RB, :] for c in range(4)]
        lg = []
        for w in range(W):
            st = HALO + base + r0 - DIL * w
            s = _tree(jnp.add, [q[c] * kv[c, st:st + RB, :] for c in range(4)])
            s = s + pltpu.roll(s, 64, 1)
            s = s + pltpu.roll(s, 32, 1)
            if row0 is not None and r0 < DIL * w:
                pos = row0 + r0 + jax.lax.broadcasted_iota(i32, (RB, 128), 0)
                s = jnp.where(pos >= DIL * w, s, -1e9 / SCALE)
            lg.append(s)
        m = _tree(jnp.maximum, lg)
        e = [jnp.exp2((l - m) * (SCALE * math.log2(math.e))) for l in lg]
        inv = _recip(_tree(jnp.add, e))
        for c in range(4):
            st = HALO + base + r0
            acc = inv * _tree(jnp.add, [e[w] * kv[4 + c, st - DIL * w:st - DIL * w + RB, :]
                                        for w in range(W)])
            if not last:
                tok = acc[0:8] if tok is None else tok + acc[0:8]
            elif c == 3:
                acc = jnp.where(zero_s[...] == 0, acc, jnp.concatenate([tok] * (RB // 8), axis=0))
            y_s[b][r0 // 2:(r0 + RB) // 2, c * 128:(c + 1) * 128] = _pk(acc)
        return None if last else pltpu.roll(tok, 1, 1)

    def ln_stage(fn, load, ref, *lead):
        for r0 in range(0, SUB, LB):
            ref[(*lead, slice(r0 // 2, (r0 + LB) // 2), slice(None))] = _pk(fn(load(r0)))

    def rows(ref, *lead):
        return lambda r: ref[(*lead, slice(r, r + LB), slice(None))]

    def ln_in(b, row0):
        ln_stage(_ln, lambda r: x_v[pl.ds(row0 + r, LB), :].astype(f32), y_s[b])

    def st_q(ctx, lo=0, hi=3):
        b, kv, base = ctx
        qkv = jnp.dot(_up(y_s[b][...]), _up(wqkv_p[:, lo * D:hi * D]), preferred_element_type=f32)
        for c in range(4 * lo, 4 * hi):
            blk = qkv[:, c * 128 - lo * D:(c + 1) * 128 - lo * D]
            if c < 4:
                q_s[b][c] = blk
            else:
                kv[c - 4, HALO + base:HALO + base + SUB, :] = blk

    def attn_out(ctx, mask_row0):
        tok = None
        for rb in range(SUB // RB):
            tok = attn_block(ctx, rb, mask_row0, tok)
        return jnp.dot(_up(y_s[ctx[0]][...]), _up(wo_p[...]), preferred_element_type=f32)

    def halo(kv, n):
        kv[:, 0:HALO, :] = kv[:, n:n + HALO, :]

    def st_o1(ctx, j, row0, slot, mask_row0=None):
        x1_s[j][slot] = x_v[pl.ds(row0, SUB), :].astype(f32) + attn_out(ctx, mask_row0)
        ln_stage(_ln_ln, rows(x1_s[j], slot), y2_s[j], slot)

    def st_o2(ctx, j, mask_row0=None):
        x_s[j][...] = x_s[j][...] + attn_out(ctx, mask_row0)
        ln_stage(_ln_ln, rows(x_s[j]), y_s[ctx[0]])

    def st_u(j, y):
        h = jax.lax.dot_general(_up(y), w1t_v[...], (((1,), (1,)), ((), ())),
                                preferred_element_type=f32) + b1_s[...]
        g_s[j][...] = _pk(_gelu(h))

    def mlp_out(j):
        return jnp.dot(_up(g_s[j][...]), w2_v[...], preferred_element_type=f32) + b2_s[...]

    def st_d1(j):
        x_s[j][...] = x1_s[j][0] + mlp_out(j)
        ln_stage(_ln, rows(x_s[j]), y_s[2 + j])
        x1_s[j][0] = x1_s[j][1]
        y2_s[j][0] = y2_s[j][1]

    def st_d2(j, row0):
        o_v[pl.ds(row0, SUB), :] = (x_s[j][...] + mlp_out(j)).astype(bf16)
        cp_out(row0).start()

    ca = [(j, kv0_s, j * SUB) for j in range(2)]
    cm = [(2 + j, kv1_s, j * SUB) for j in range(2)]
    cb = [(2 + j, kv0_s, TM + j * SUB) for j in range(2)]

    def perm_cols(t):
        lane = jax.lax.broadcasted_iota(i32, (PR, 128), 1)
        for r in range(D // 2 // PR):
            src = [pltpu.bitcast(wqkv_v[t, 2 * r * PR:2 * (r + 1) * PR, c * 128:(c + 1) * 128], u32)
                   for c in range(4)]
            for j in range(4):
                mixed = _sel4(((lane // 4) % 4 - j) % 4, src)
                idx = (lane % 8) * 16 + (((lane // 8) + j) % 4) * 4 + lane // 32
                wqkv_p[r * PR:(r + 1) * PR, t * D + j * 128:t * D + (j + 1) * 128] = (
                    jnp.take_along_axis(mixed, idx, axis=1))

    def perm_wo():
        dhi = (jax.lax.broadcasted_iota(i32, (64, D), 0) // 2) % 4
        src = [pltpu.bitcast(wo_v[c * 128:(c + 1) * 128, :], u32) for c in range(4)]
        for j in range(4):
            mixed = _sel4((dhi - j) % 4, src)
            wo_p[j * 64:(j + 1) * 64, :] = _pk(
                jnp.dot(_up(pt_s[j]), _up(mixed), preferred_element_type=f32))

    ops = {
        'L0': lambda: (ln_in(0, 0), ln_in(1, SUB)),
        'L1': lambda: (ln_in(2, TM), ln_in(3, TM + SUB)),
        'W': perm_wo,
        'oX0': lambda: st_o1(ca[0], 0, 0, 0, mask_row0=0),
        'oY0': lambda: st_o1(ca[1], 1, SUB, 0),
        'oX1': lambda: st_o1(cb[0], 0, TM, 1),
        'oY1': lambda: st_o1(cb[1], 1, TM + SUB, 1),
    }
    for t, nm in enumerate('qkv'):
        ops['P' + nm] = functools.partial(perm_cols, t)
        for j, ch in enumerate('XY'):
            ops[nm + ch + '0'] = functools.partial(st_q, ca[j], t, t + 1)
            ops[nm + ch + '1'] = functools.partial(st_q, cb[j], t, t + 1)
    for name in ('!x0 L0 !Wq Pq qX0 !Wk Pk qY0 kX0 !Wv Pv kY0 vX0 !wo !x1 L1 vY0 W qX1 oX0 kX1 vX1 '
                 'oY0 qY1 kY1 vY1 oX1 oY1').split():
        if name[0] == '!':
            cps[name[1:]].wait()
        else:
            ops[name]()
    halo(kv0_s, LA * TM)
    cps['b1'].wait()
    cps['b2'].wait()
    b1_s[...] = b1_v[...].astype(f32).reshape(1, F)
    b2_s[...] = b2_v[...].astype(f32).reshape(1, D)
    cps['w1'].wait()
    cps['w2'].wait()
    cps['x2'].wait()
    cp_xr.start()

    def steady(k, ahead):
        rx = pl.multiple_of(k * TM, TM)
        ry = pl.multiple_of(rx + SUB, SUB)
        rn = pl.multiple_of(rx + LA * TM, TM)
        rm = pl.multiple_of(rn + SUB, SUB)
        st_u(0, y2_s[0][0])
        if ahead:
            ln_in(0, rn)
            st_q(ca[0])
        st_d1(0)
        st_u(1, y2_s[1][0])
        if ahead:
            st_o1(ca[0], 0, rn, 1)
        st_q(cm[0])
        st_d1(1)
        st_o2(cm[0], 0, mask_row0=rx if ahead else None)
        st_q(cm[1])
        st_u(0, y_s[2][...])
        st_o2(cm[1], 1)
        halo(kv1_s, TM)
        if ahead:
            ln_in(1, rm)
            st_q(ca[1])
        st_d2(0, rx)
        st_u(1, y_s[3][...])
        if ahead:
            st_o1(ca[1], 1, rm, 1)
            halo(kv0_s, TM)
        st_d2(1, ry)

    def body1(k, carry):
        @pl.when(k == 1)
        def _():
            cp_xr.wait()
        steady(k, True)
        return carry

    def body2(k, carry):
        steady(k, False)
        return carry

    jax.lax.fori_loop(0, NIT - LA, body1, 0)
    jax.lax.fori_loop(NIT - LA, NIT, body2, 0)
    for t in range(S // SUB):
        cp_out(t * SUB).wait()


@jax.jit
def pallas_interleave_layers__sliding_local_dilated__mixer_channel_mlp__prompt_kernel(
    A_x: jax.Array,
    A_wqkv: jax.Array,
    A_wo: jax.Array,
    B_x: jax.Array,
    B_w1: jax.Array,
    B_b1: jax.Array,
    B_w2: jax.Array,
    B_b2: jax.Array,
):
    del B_x
    hbm = pl.BlockSpec(memory_space=pl.ANY)
    out = pl.pallas_call(
        _kernel,
        in_specs=[hbm] * 7,
        out_specs=hbm,
        out_shape=jax.ShapeDtypeStruct((S, D), bf16),
        scratch_shapes=[
            pltpu.VMEM((S, D), bf16),
            pltpu.VMEM((S, D), bf16),
            pltpu.VMEM((3, D, D), bf16),
            pltpu.VMEM((D, D), bf16),
            pltpu.VMEM((F, D), bf16),
            pltpu.VMEM((F, D), bf16),
            pltpu.VMEM((F,), bf16),
            pltpu.VMEM((D,), bf16),
            pltpu.VMEM((D // 2, 3 * D), u32),
            pltpu.VMEM((D // 2, D), u32),
            pltpu.VMEM((4, 64, 128), u32),
            pltpu.VMEM((RB, 128), i32),
            pltpu.VMEM((1, F), f32),
            pltpu.VMEM((1, D), f32),
            pltpu.VMEM((8, LA * TM + HALO + KPAD, 128), f32),
            pltpu.VMEM((8, TM + HALO + KPAD, 128), f32),
            pltpu.SemaphoreType.DMA((12,)),
            pltpu.SemaphoreType.DMA,
        ] + [pltpu.VMEM((SUB, D), f32) for _ in range(2)]
          + [pltpu.VMEM((SUB // 2, F), u32) for _ in range(2)]
          + [pltpu.VMEM((LA, SUB, D), f32) for _ in range(2)]
          + [pltpu.VMEM((LA, SUB // 2, D), u32) for _ in range(2)]
          + [pltpu.VMEM((SUB // 2, D), u32) for _ in range(4)]
          + [pltpu.VMEM((4, SUB, 128), f32) for _ in range(4)],
        compiler_params=pltpu.CompilerParams(vmem_limit_bytes=64 * 1024 * 1024),
    )(A_x.reshape(S, D), A_wqkv, A_wo, B_w1.T, B_b1, B_w2, B_b2)
    return out.reshape(1, S, D)
```

```python
import functools
import math

import jax
import jax.numpy as jnp
import jax.experimental.pallas as pl
import jax.experimental.pallas.tpu as pltpu

S, D, F = 2048, 512, 1376
H, DH, W, DIL = 32, 16, 8, 2
EPS = 1e-5
SCALE = DH ** -0.5
HALO = 16
SUB = 128
TM = 2 * SUB
NIT = S // TM
LA = 2
RB = 16
LB = 32
PR = 64
bf16, f32, u32, i32 = jnp.bfloat16, jnp.float32, jnp.uint32, jnp.int32


def _stats(x):
    m = jnp.sum(x, axis=-1, keepdims=True) * (1.0 / D)
    xc = x - m
    v = jnp.sum(xc * xc, axis=-1, keepdims=True) * (1.0 / D)
    return xc, v


def _ln(x):
    xc, v = _stats(x)
    return xc * jax.lax.rsqrt(v + EPS)


def _ln_ln(x):
    xc, v = _stats(x)
    return xc * jax.lax.rsqrt(v * (1.0 + EPS) + EPS * EPS)


def _gelu(h):
    c = math.sqrt(2.0 / math.pi)
    u = h * (c + (c * 0.044715) * (h * h))
    hh = 0.5 * h
    return hh + hh * jnp.tanh(u)


def _tree(op, xs):
    xs = list(xs)
    while len(xs) > 1:
        nxt = [op(xs[k], xs[k + 1]) for k in range(0, len(xs) - 1, 2)]
        if len(xs) % 2:
            nxt.append(xs[-1])
        xs = nxt
    return xs[0]


def _recip(d):
    r = pl.reciprocal(d, approx=True)
    return r * (2.0 - d * r)


def _pk(v):
    return pltpu.bitcast(v.astype(bf16), u32)


def _up(v):
    return pltpu.bitcast(v, bf16)


def _sel4(sel, vals):
    return jnp.where(sel < 2, jnp.where(sel == 0, vals[0], vals[1]),
                     jnp.where(sel == 2, vals[2], vals[3]))


def _kernel(x_hbm, wqkv_hbm, wo_hbm, w1t_hbm, b1_hbm, w2_hbm, b2_hbm, o_hbm,
            x_v, o_v, wqkv_v, wo_v, w1t_v, w2_v, b1_v, b2_v,
            wqkv_p, wo_p, pt_s, zero_s, b1_s, b2_s, kv0_s, kv1_s, sem, osem, *bufs):
    x_s = bufs[0:2]
    g_s = bufs[2:4]
    x1_s = bufs[4:6]
    y2_s = bufs[6:8]
    y_s = bufs[8:12]
    q_s = bufs[12:16]

    def cp_x(lo, hi, s):
        return pltpu.make_async_copy(x_hbm.at[lo:hi], x_v.at[lo:hi], sem.at[s])

    cps = {
        'x0': cp_x(0, TM, 0),
        'Wq': pltpu.make_async_copy(wqkv_hbm.at[:, 0:D], wqkv_v.at[0], sem.at[1]),
        'Wk': pltpu.make_async_copy(wqkv_hbm.at[:, D:2 * D], wqkv_v.at[1], sem.at[2]),
        'Wv': pltpu.make_async_copy(wqkv_hbm.at[:, 2 * D:3 * D], wqkv_v.at[2], sem.at[3]),
        'wo': pltpu.make_async_copy(wo_hbm, wo_v, sem.at[4]),
        'x1': cp_x(TM, LA * TM, 5),
        'b1': pltpu.make_async_copy(b1_hbm, b1_v, sem.at[6]),
        'b2': pltpu.make_async_copy(b2_hbm, b2_v, sem.at[7]),
        'w1': pltpu.make_async_copy(w1t_hbm, w1t_v, sem.at[8]),
        'w2': pltpu.make_async_copy(w2_hbm, w2_v, sem.at[9]),
        'x2': cp_x(LA * TM, (LA + 1) * TM, 10),
    }
    cp_xr = cp_x((LA + 1) * TM, S, 11)

    def cp_out(row, n):
        return pltpu.make_async_copy(o_v.at[pl.ds(row, n)], o_hbm.at[pl.ds(row, n)], osem)

    for cp in cps.values():
        cp.start()

    kv0_s[:, 0:HALO, :] = jnp.zeros((8, HALO, 128), f32)
    kv1_s[:, 0:HALO, :] = jnp.zeros((8, HALO, 128), f32)
    zero_s[...] = jnp.zeros(zero_s.shape, i32)

    src_id = jax.lax.broadcasted_iota(i32, (128, 128), 1)
    dst_id = jax.lax.broadcasted_iota(i32, (128, 128), 0)
    for j in range(4):
        hit = dst_id == (src_id % 4) * 32 + (((src_id // 4) % 4 - j) % 4) * 8 + src_id // 16
        pt_s[j] = _pk(jnp.where(hit, 1.0, 0.0))

    def attn_block(ctx, rb, row0, tok):
        b, kv, base = ctx
        r0 = rb * RB
        last = rb == SUB // RB - 1
        q = [q_s[b][c, r0:r0 + RB, :] for c in range(4)]
        lg = []
        for w in range(W):
            st = HALO + base + r0 - DIL * w
            s = _tree(jnp.add, [q[c] * kv[c, st:st + RB, :] for c in range(4)])
            s = s + pltpu.roll(s, 64, 1)
            s = s + pltpu.roll(s, 32, 1)
            if row0 is not None and r0 < DIL * w:
                pos = row0 + r0 + jax.lax.broadcasted_iota(i32, (RB, 128), 0)
                s = jnp.where(pos >= DIL * w, s, -1e9 / SCALE)
            lg.append(s)
        m = _tree(jnp.maximum, lg)
        e = [jnp.exp2((l - m) * (SCALE * math.log2(math.e))) for l in lg]
        inv = _recip(_tree(jnp.add, e))
        for c in range(4):
            st = HALO + base + r0
            acc = inv * _tree(jnp.add, [e[w] * kv[4 + c, st - DIL * w:st - DIL * w + RB, :]
                                        for w in range(W)])
            if not last:
                tok = acc[0:8] if tok is None else tok + acc[0:8]
            elif c == 3:
                acc = jnp.where(zero_s[...] == 0, acc, jnp.concatenate([tok] * (RB // 8), axis=0))
            y_s[b][r0 // 2:(r0 + RB) // 2, c * 128:(c + 1) * 128] = _pk(acc)
        return None if last else pltpu.roll(tok, 1, 1)

    def ln_stage(fn, load, ref, *lead):
        for r0 in range(0, SUB, LB):
            ref[(*lead, slice(r0 // 2, (r0 + LB) // 2), slice(None))] = _pk(fn(load(r0)))

    def rows(ref, *lead):
        return lambda r: ref[(*lead, slice(r, r + LB), slice(None))]

    def ln_in(b, row0):
        ln_stage(_ln, lambda r: x_v[pl.ds(row0 + r, LB), :].astype(f32), y_s[b])

    def st_q(ctx, lo=0, hi=3):
        b, kv, base = ctx
        qkv = jnp.dot(_up(y_s[b][...]), _up(wqkv_p[:, lo * D:hi * D]), preferred_element_type=f32)
        for c in range(4 * lo, 4 * hi):
            blk = qkv[:, c * 128 - lo * D:(c + 1) * 128 - lo * D]
            if c < 4:
                q_s[b][c] = blk
            else:
                kv[c - 4, HALO + base:HALO + base + SUB, :] = blk

    def attention(ctx, mask_row0):
        tok = None
        for rb in range(SUB // RB):
            tok = attn_block(ctx, rb, mask_row0, tok)

    def out_proj(ctx, lo=0, n=SUB):
        return jnp.dot(_up(y_s[ctx[0]][lo // 2:(lo + n) // 2, :]), _up(wo_p[...]),
                       preferred_element_type=f32)

    def halo(kv, n):
        kv[:, 0:HALO, :] = kv[:, n:n + HALO, :]

    def st_o1(ctx, j, row0, slot, mask_row0=None, parts=1):
        attention(ctx, mask_row0)
        n = SUB // parts
        for lo in range(0, SUB, n):
            x1_s[j][slot, lo:lo + n, :] = (x_v[pl.ds(row0 + lo, n), :].astype(f32)
                                           + out_proj(ctx, lo, n))
        ln_stage(_ln_ln, rows(x1_s[j], slot), y2_s[j], slot)

    def st_o2(ctx, j, mask_row0=None):
        attention(ctx, mask_row0)
        x_s[j][...] = x_s[j][...] + out_proj(ctx)
        ln_stage(_ln_ln, rows(x_s[j]), y_s[ctx[0]])

    def st_u(j, y):
        h = jax.lax.dot_general(_up(y), w1t_v[...], (((1,), (1,)), ((), ())),
                                preferred_element_type=f32) + b1_s[...]
        g_s[j][...] = _pk(_gelu(h))

    def mlp_out(j, lo=0, n=SUB):
        return jnp.dot(_up(g_s[j][lo // 2:(lo + n) // 2, :]), w2_v[...],
                       preferred_element_type=f32) + b2_s[...]

    def st_d1(j):
        x_s[j][...] = x1_s[j][0] + mlp_out(j)
        ln_stage(_ln, rows(x_s[j]), y_s[2 + j])
        x1_s[j][0] = x1_s[j][1]
        y2_s[j][0] = y2_s[j][1]

    def st_d2(j, row0, parts=1):
        n = SUB // parts
        for lo in range(0, SUB, n):
            r = pl.multiple_of(row0 + lo, n)
            o_v[pl.ds(r, n), :] = (x_s[j][lo:lo + n, :] + mlp_out(j, lo, n)).astype(bf16)
            cp_out(r, n).start()

    ca = [(j, kv0_s, j * SUB) for j in range(2)]
    cm = [(2 + j, kv1_s, j * SUB) for j in range(2)]
    cb = [(2 + j, kv0_s, TM + j * SUB) for j in range(2)]

    def perm_cols(t):
        lane = jax.lax.broadcasted_iota(i32, (PR, 128), 1)
        for r in range(D // 2 // PR):
            src = [pltpu.bitcast(wqkv_v[t, 2 * r * PR:2 * (r + 1) * PR, c * 128:(c + 1) * 128], u32)
                   for c in range(4)]
            for j in range(4):
                mixed = _sel4(((lane // 4) % 4 - j) % 4, src)
                idx = (lane % 8) * 16 + (((lane // 8) + j) % 4) * 4 + lane // 32
                wqkv_p[r * PR:(r + 1) * PR, t * D + j * 128:t * D + (j + 1) * 128] = (
                    jnp.take_along_axis(mixed, idx, axis=1))

    def perm_wo():
        dhi = (jax.lax.broadcasted_iota(i32, (64, D), 0) // 2) % 4
        src = [pltpu.bitcast(wo_v[c * 128:(c + 1) * 128, :], u32) for c in range(4)]
        for j in range(4):
            mixed = _sel4((dhi - j) % 4, src)
            wo_p[j * 64:(j + 1) * 64, :] = _pk(
                jnp.dot(_up(pt_s[j]), _up(mixed), preferred_element_type=f32))

    ops = {
        'L0': lambda: (ln_in(0, 0), ln_in(1, SUB)),
        'L1': lambda: (ln_in(2, TM), ln_in(3, TM + SUB)),
        'W': perm_wo,
        'oX0': lambda: st_o1(ca[0], 0, 0, 0, mask_row0=0),
        'oY0': lambda: st_o1(ca[1], 1, SUB, 0),
        'oX1': lambda: st_o1(cb[0], 0, TM, 1),
        'oY1': lambda: st_o1(cb[1], 1, TM + SUB, 1, parts=4),
    }
    for t, nm in enumerate('qkv'):
        ops['P' + nm] = functools.partial(perm_cols, t)
        for j, ch in enumerate('XY'):
            ops[nm + ch + '0'] = functools.partial(st_q, ca[j], t, t + 1)
            ops[nm + ch + '1'] = functools.partial(st_q, cb[j], t, t + 1)
    for name in ('!x0 L0 !Wq Pq qX0 !Wk Pk qY0 kX0 !Wv Pv kY0 vX0 !wo !x1 L1 vY0 W qX1 oX0 kX1 vX1 '
                 'oY0 qY1 kY1 vY1 oX1 oY1').split():
        if name[0] == '!':
            cps[name[1:]].wait()
        else:
            ops[name]()
    halo(kv0_s, LA * TM)
    cps['b1'].wait()
    cps['b2'].wait()
    b1_s[...] = b1_v[...].astype(f32).reshape(1, F)
    b2_s[...] = b2_v[...].astype(f32).reshape(1, D)
    cps['w1'].wait()
    cps['w2'].wait()
    cps['x2'].wait()
    cp_xr.start()

    def steady(k, ahead):
        rx = pl.multiple_of(k * TM, TM)
        ry = pl.multiple_of(rx + SUB, SUB)
        rn = pl.multiple_of(rx + LA * TM, TM)
        rm = pl.multiple_of(rn + SUB, SUB)
        st_u(0, y2_s[0][0])
        if ahead:
            ln_in(0, rn)
            st_q(ca[0])
        st_d1(0)
        st_u(1, y2_s[1][0])
        if ahead:
            st_o1(ca[0], 0, rn, 1)
        st_q(cm[0])
        st_d1(1)
        st_o2(cm[0], 0, mask_row0=rx if ahead else None)
        st_q(cm[1])
        st_u(0, y_s[2][...])
        st_o2(cm[1], 1)
        halo(kv1_s, TM)
        if ahead:
            ln_in(1, rm)
            st_q(ca[1])
        st_d2(0, rx)
        st_u(1, y_s[3][...])
        if ahead:
            st_o1(ca[1], 1, rm, 1)
            halo(kv0_s, TM)
        st_d2(1, ry, parts=1 if ahead else 2)

    def body1(k, carry):
        @pl.when(k == 1)
        def _():
            cp_xr.wait()
        steady(k, True)
        return carry

    def body2(k, carry):
        steady(k, False)
        return carry

    jax.lax.fori_loop(0, NIT - LA, body1, 0)
    jax.lax.fori_loop(NIT - LA, NIT, body2, 0)
    for k in range(NIT):
        cp_out(k * TM, SUB).wait()
        n = SUB if k < NIT - LA else SUB // 2
        for lo in range(0, SUB, n):
            cp_out(k * TM + SUB + lo, n).wait()


@jax.jit
def pallas_interleave_layers__sliding_local_dilated__mixer_channel_mlp__prompt_kernel(
    A_x: jax.Array,
    A_wqkv: jax.Array,
    A_wo: jax.Array,
    B_x: jax.Array,
    B_w1: jax.Array,
    B_b1: jax.Array,
    B_w2: jax.Array,
    B_b2: jax.Array,
):
    del B_x
    hbm = pl.BlockSpec(memory_space=pl.ANY)
    out = pl.pallas_call(
        _kernel,
        in_specs=[hbm] * 7,
        out_specs=hbm,
        out_shape=jax.ShapeDtypeStruct((S, D), bf16),
        scratch_shapes=[
            pltpu.VMEM((S, D), bf16),
            pltpu.VMEM((S, D), bf16),
            pltpu.VMEM((3, D, D), bf16),
            pltpu.VMEM((D, D), bf16),
            pltpu.VMEM((F, D), bf16),
            pltpu.VMEM((F, D), bf16),
            pltpu.VMEM((F,), bf16),
            pltpu.VMEM((D,), bf16),
            pltpu.VMEM((D // 2, 3 * D), u32),
            pltpu.VMEM((D // 2, D), u32),
            pltpu.VMEM((4, 64, 128), u32),
            pltpu.VMEM((RB, 128), i32),
            pltpu.VMEM((1, F), f32),
            pltpu.VMEM((1, D), f32),
            pltpu.VMEM((8, LA * TM + HALO, 128), f32),
            pltpu.VMEM((8, TM + HALO, 128), f32),
            pltpu.SemaphoreType.DMA((12,)),
            pltpu.SemaphoreType.DMA,
        ] + [pltpu.VMEM((SUB, D), f32) for _ in range(2)]
          + [pltpu.VMEM((SUB // 2, F), u32) for _ in range(2)]
          + [pltpu.VMEM((LA, SUB, D), f32) for _ in range(2)]
          + [pltpu.VMEM((LA, SUB // 2, D), u32) for _ in range(2)]
          + [pltpu.VMEM((SUB // 2, D), u32) for _ in range(4)]
          + [pltpu.VMEM((4, SUB, 128), f32) for _ in range(4)],
        compiler_params=pltpu.CompilerParams(vmem_limit_bytes=64 * 1024 * 1024),
    )(A_x.reshape(S, D), A_wqkv, A_wo, B_w1.T, B_b1, B_w2, B_b2)
    return out.reshape(1, S, D)
```

```python
import functools
import math

import jax
import jax.numpy as jnp
import jax.experimental.pallas as pl
import jax.experimental.pallas.tpu as pltpu

S, D, F = 2048, 512, 1376
H, DH, W, DIL = 32, 16, 8, 2
EPS = 1e-5
SCALE = DH ** -0.5
HALO = 16
SUB = 128
TM = 2 * SUB
NIT = S // TM
LA = 2
RB = 16
LB = 32
PR = 64
bf16, f32, u32, i32 = jnp.bfloat16, jnp.float32, jnp.uint32, jnp.int32


def _ln(x):
    m = jnp.sum(x, axis=-1, keepdims=True) * (1.0 / D)
    xc = x - m
    v = jnp.sum(xc * xc, axis=-1, keepdims=True) * (1.0 / D)
    return xc * jax.lax.rsqrt(v + EPS)


def _ln_ln(x):
    return _ln(_ln(x))


def _gelu(h):
    c = math.sqrt(2.0 / math.pi)
    u = h * (c + (c * 0.044715) * (h * h))
    hh = 0.5 * h
    return hh + hh * jnp.tanh(u)


def _tree(op, xs):
    xs = list(xs)
    while len(xs) > 1:
        nxt = [op(xs[k], xs[k + 1]) for k in range(0, len(xs) - 1, 2)]
        if len(xs) % 2:
            nxt.append(xs[-1])
        xs = nxt
    return xs[0]


def _recip(d):
    r = pl.reciprocal(d, approx=True)
    return r * (2.0 - d * r)


def _pk(v):
    return pltpu.bitcast(v.astype(bf16), u32)


def _up(v):
    return pltpu.bitcast(v, bf16)


def _sel4(sel, vals):
    return jnp.where(sel < 2, jnp.where(sel == 0, vals[0], vals[1]),
                     jnp.where(sel == 2, vals[2], vals[3]))


def _kernel(x_hbm, wqkv_hbm, wo_hbm, w1t_hbm, b1_hbm, w2_hbm, b2_hbm, o_hbm,
            x_v, o_v, wqkv_v, wo_v, w1t_v, w2_v, b1_v, b2_v,
            wqkv_p, wo_p, pt_s, zero_s, b1_s, b2_s, kv0_s, kv1_s, sem, osem, *bufs):
    x_s = bufs[0:2]
    g_s = bufs[2:4]
    x1_s = bufs[4:6]
    y2_s = bufs[6:8]
    y_s = bufs[8:12]
    q_s = bufs[12:16]

    def cp_x(lo, hi, s):
        return pltpu.make_async_copy(x_hbm.at[lo:hi], x_v.at[lo:hi], sem.at[s])

    cps = {
        'x0': cp_x(0, TM, 0),
        'Wq': pltpu.make_async_copy(wqkv_hbm.at[:, 0:D], wqkv_v.at[0], sem.at[1]),
        'Wk': pltpu.make_async_copy(wqkv_hbm.at[:, D:2 * D], wqkv_v.at[1], sem.at[2]),
        'Wv': pltpu.make_async_copy(wqkv_hbm.at[:, 2 * D:3 * D], wqkv_v.at[2], sem.at[3]),
        'wo': pltpu.make_async_copy(wo_hbm, wo_v, sem.at[4]),
        'x1': cp_x(TM, LA * TM, 5),
        'b1': pltpu.make_async_copy(b1_hbm, b1_v, sem.at[6]),
        'b2': pltpu.make_async_copy(b2_hbm, b2_v, sem.at[7]),
        'w1': pltpu.make_async_copy(w1t_hbm, w1t_v, sem.at[8]),
        'w2': pltpu.make_async_copy(w2_hbm, w2_v, sem.at[9]),
        'x2': cp_x(LA * TM, (LA + 1) * TM, 10),
    }
    cp_xr = cp_x((LA + 1) * TM, S, 11)

    def cp_out(row, n):
        return pltpu.make_async_copy(o_v.at[pl.ds(row, n)], o_hbm.at[pl.ds(row, n)], osem)

    for cp in cps.values():
        cp.start()

    kv0_s[:, 0:HALO, :] = jnp.zeros((8, HALO, 128), f32)
    kv1_s[:, 0:HALO, :] = jnp.zeros((8, HALO, 128), f32)
    zero_s[...] = jnp.zeros(zero_s.shape, i32)

    src_id = jax.lax.broadcasted_iota(i32, (128, 128), 1)
    dst_id = jax.lax.broadcasted_iota(i32, (128, 128), 0)
    for j in range(4):
        hit = dst_id == (src_id % 4) * 32 + (((src_id // 4) % 4 - j) % 4) * 8 + src_id // 16
        pt_s[j] = _pk(jnp.where(hit, 1.0, 0.0))

    def attn_block(ctx, rb, row0, tok):
        b, kv, base = ctx
        r0 = rb * RB
        last = rb == SUB // RB - 1
        q = [q_s[b][c, r0:r0 + RB, :] for c in range(4)]
        lg = []
        for w in range(W):
            st = HALO + base + r0 - DIL * w
            s = _tree(jnp.add, [q[c] * kv[c, st:st + RB, :] for c in range(4)])
            s = s + pltpu.roll(s, 64, 1)
            s = s + pltpu.roll(s, 32, 1)
            if row0 is not None and r0 < DIL * w:
                pos = row0 + r0 + jax.lax.broadcasted_iota(i32, (RB, 128), 0)
                s = jnp.where(pos >= DIL * w, s, -1e9 / SCALE)
            lg.append(s)
        m = _tree(jnp.maximum, lg)
        e = [jnp.exp2((l - m) * (SCALE * math.log2(math.e))) for l in lg]
        inv = _recip(_tree(jnp.add, e))
        for c in range(4):
            st = HALO + base + r0
            acc = inv * _tree(jnp.add, [e[w] * kv[4 + c, st - DIL * w:st - DIL * w + RB, :]
                                        for w in range(W)])
            if not last:
                tok = acc[0:8] if tok is None else tok + acc[0:8]
            elif c == 3:
                acc = jnp.where(zero_s[...] == 0, acc, jnp.concatenate([tok] * (RB // 8), axis=0))
            y_s[b][r0 // 2:(r0 + RB) // 2, c * 128:(c + 1) * 128] = _pk(acc)
        return None if last else pltpu.roll(tok, 1, 1)

    def ln_stage(fn, load, ref):
        for r0 in range(0, SUB, LB):
            ref[r0 // 2:(r0 + LB) // 2, :] = _pk(fn(load(r0)))

    def rows(ref, *lead):
        return lambda r: ref[(*lead, slice(r, r + LB), slice(None))]

    def ln_in(b, row0):
        ln_stage(_ln, lambda r: x_v[pl.ds(row0 + r, LB), :].astype(f32), y_s[b])

    def st_q(ctx, lo=0, hi=3):
        b, kv, base = ctx
        qkv = jnp.dot(_up(y_s[b][...]), _up(wqkv_p[:, lo * D:hi * D]), preferred_element_type=f32)
        for c in range(4 * lo, 4 * hi):
            blk = qkv[:, c * 128 - lo * D:(c + 1) * 128 - lo * D]
            if c < 4:
                q_s[b][c] = blk
            else:
                kv[c - 4, HALO + base:HALO + base + SUB, :] = blk

    def attention(ctx, mask_row0):
        tok = None
        for rb in range(SUB // RB):
            tok = attn_block(ctx, rb, mask_row0, tok)

    def out_proj(ctx, lo=0, n=SUB):
        return jnp.dot(_up(y_s[ctx[0]][lo // 2:(lo + n) // 2, :]), _up(wo_p[...]),
                       preferred_element_type=f32)

    def halo(kv, n):
        kv[:, 0:HALO, :] = kv[:, n:n + HALO, :]

    def st_o1(ctx, j, row0, slot, mask_row0=None, parts=1):
        attention(ctx, mask_row0)
        n = SUB // parts
        for lo in range(0, SUB, n):
            x1_s[j][slot, lo:lo + n, :] = (x_v[pl.ds(row0 + lo, n), :].astype(f32)
                                           + out_proj(ctx, lo, n))

    def ln2(j, slot):
        ln_stage(_ln_ln, rows(x1_s[j], slot), y2_s[j])

    def st_o2(ctx, j, mask_row0=None):
        attention(ctx, mask_row0)
        x_s[j][...] = x_s[j][...] + out_proj(ctx)
        ln_stage(_ln_ln, rows(x_s[j]), y_s[ctx[0]])

    def st_u(j, y):
        h = jax.lax.dot_general(_up(y), w1t_v[...], (((1,), (1,)), ((), ())),
                                preferred_element_type=f32) + b1_s[...]
        g_s[j][...] = _pk(_gelu(h))

    def mlp_out(j, lo=0, n=SUB):
        return jnp.dot(_up(g_s[j][lo // 2:(lo + n) // 2, :]), w2_v[...],
                       preferred_element_type=f32) + b2_s[...]

    def st_d1(j):
        x_s[j][...] = x1_s[j][0] + mlp_out(j)
        ln_stage(_ln, rows(x_s[j]), y_s[2 + j])
        x1_s[j][0] = x1_s[j][1]

    def st_d2(j, row0, parts=1):
        n = SUB // parts
        for lo in range(0, SUB, n):
            r = pl.multiple_of(row0 + lo, n)
            o_v[pl.ds(r, n), :] = (x_s[j][lo:lo + n, :] + mlp_out(j, lo, n)).astype(bf16)
            cp_out(r, n).start()

    ca = [(j, kv0_s, j * SUB) for j in range(2)]
    cm = [(2 + j, kv1_s, j * SUB) for j in range(2)]
    cb = [(2 + j, kv0_s, TM + j * SUB) for j in range(2)]

    def perm_cols(t):
        lane = jax.lax.broadcasted_iota(i32, (PR, 128), 1)
        for r in range(D // 2 // PR):
            src = [pltpu.bitcast(wqkv_v[t, 2 * r * PR:2 * (r + 1) * PR, c * 128:(c + 1) * 128], u32)
                   for c in range(4)]
            for j in range(4):
                mixed = _sel4(((lane // 4) % 4 - j) % 4, src)
                idx = (lane % 8) * 16 + (((lane // 8) + j) % 4) * 4 + lane // 32
                wqkv_p[r * PR:(r + 1) * PR, t * D + j * 128:t * D + (j + 1) * 128] = (
                    jnp.take_along_axis(mixed, idx, axis=1))

    def perm_wo():
        dhi = (jax.lax.broadcasted_iota(i32, (64, D), 0) // 2) % 4
        src = [pltpu.bitcast(wo_v[c * 128:(c + 1) * 128, :], u32) for c in range(4)]
        for j in range(4):
            mixed = _sel4((dhi - j) % 4, src)
            wo_p[j * 64:(j + 1) * 64, :] = _pk(
                jnp.dot(_up(pt_s[j]), _up(mixed), preferred_element_type=f32))

    ops = {
        'L0': lambda: (ln_in(0, 0), ln_in(1, SUB)),
        'L1': lambda: (ln_in(2, TM), ln_in(3, TM + SUB)),
        'W': perm_wo,
        'oX0': lambda: (st_o1(ca[0], 0, 0, 0, mask_row0=0), ln2(0, 0)),
        'oY0': lambda: (st_o1(ca[1], 1, SUB, 0), ln2(1, 0)),
        'oX1': lambda: st_o1(cb[0], 0, TM, 1),
        'oY1': lambda: st_o1(cb[1], 1, TM + SUB, 1, parts=4),
    }
    for t, nm in enumerate('qkv'):
        ops['P' + nm] = functools.partial(perm_cols, t)
        for j, ch in enumerate('XY'):
            ops[nm + ch + '0'] = functools.partial(st_q, ca[j], t, t + 1)
            ops[nm + ch + '1'] = functools.partial(st_q, cb[j], t, t + 1)
    for name in ('!x0 L0 !Wq Pq qX0 !Wk Pk qY0 kX0 !Wv Pv kY0 vX0 !wo !x1 L1 vY0 W qX1 oX0 kX1 vX1 '
                 'oY0 qY1 kY1 vY1 oX1 oY1').split():
        if name[0] == '!':
            cps[name[1:]].wait()
        else:
            ops[name]()
    halo(kv0_s, LA * TM)
    cps['b1'].wait()
    cps['b2'].wait()
    b1_s[...] = b1_v[...].astype(f32).reshape(1, F)
    b2_s[...] = b2_v[...].astype(f32).reshape(1, D)
    cps['w1'].wait()
    cps['w2'].wait()
    cps['x2'].wait()
    cp_xr.start()

    def steady(k, ahead):
        rx = pl.multiple_of(k * TM, TM)
        ry = pl.multiple_of(rx + SUB, SUB)
        rn = pl.multiple_of(rx + LA * TM, TM)
        rm = pl.multiple_of(rn + SUB, SUB)
        st_u(0, y2_s[0][...])
        ln2(0, 1)
        if ahead:
            ln_in(0, rn)
            st_q(ca[0])
        st_d1(0)
        st_u(1, y2_s[1][...])
        ln2(1, 1)
        if ahead:
            st_o1(ca[0], 0, rn, 1)
        st_q(cm[0])
        st_d1(1)
        st_o2(cm[0], 0, mask_row0=rx if ahead else None)
        st_q(cm[1])
        st_u(0, y_s[2][...])
        st_o2(cm[1], 1)
        halo(kv1_s, TM)
        if ahead:
            ln_in(1, rm)
            st_q(ca[1])
        st_d2(0, rx)
        st_u(1, y_s[3][...])
        if ahead:
            st_o1(ca[1], 1, rm, 1)
            halo(kv0_s, TM)
        st_d2(1, ry, parts=1 if ahead else 2)

    def body1(k, carry):
        @pl.when(k == 1)
        def _():
            cp_xr.wait()
        steady(k, True)
        return carry

    def body2(k, carry):
        steady(k, False)
        return carry

    jax.lax.fori_loop(0, NIT - LA, body1, 0)
    jax.lax.fori_loop(NIT - LA, NIT, body2, 0)
    for k in range(NIT):
        cp_out(k * TM, SUB).wait()
        n = SUB if k < NIT - LA else SUB // 2
        for lo in range(0, SUB, n):
            cp_out(k * TM + SUB + lo, n).wait()


@jax.jit
def pallas_interleave_layers__sliding_local_dilated__mixer_channel_mlp__prompt_kernel(
    A_x: jax.Array,
    A_wqkv: jax.Array,
    A_wo: jax.Array,
    B_x: jax.Array,
    B_w1: jax.Array,
    B_b1: jax.Array,
    B_w2: jax.Array,
    B_b2: jax.Array,
):
    del B_x
    hbm = pl.BlockSpec(memory_space=pl.ANY)
    out = pl.pallas_call(
        _kernel,
        in_specs=[hbm] * 7,
        out_specs=hbm,
        out_shape=jax.ShapeDtypeStruct((S, D), bf16),
        scratch_shapes=[
            pltpu.VMEM((S, D), bf16),
            pltpu.VMEM((S, D), bf16),
            pltpu.VMEM((3, D, D), bf16),
            pltpu.VMEM((D, D), bf16),
            pltpu.VMEM((F, D), bf16),
            pltpu.VMEM((F, D), bf16),
            pltpu.VMEM((F,), bf16),
            pltpu.VMEM((D,), bf16),
            pltpu.VMEM((D // 2, 3 * D), u32),
            pltpu.VMEM((D // 2, D), u32),
            pltpu.VMEM((4, 64, 128), u32),
            pltpu.VMEM((RB, 128), i32),
            pltpu.VMEM((1, F), f32),
            pltpu.VMEM((1, D), f32),
            pltpu.VMEM((8, LA * TM + HALO, 128), f32),
            pltpu.VMEM((8, TM + HALO, 128), f32),
            pltpu.SemaphoreType.DMA((12,)),
            pltpu.SemaphoreType.DMA,
        ] + [pltpu.VMEM((SUB, D), f32) for _ in range(2)]
          + [pltpu.VMEM((SUB // 2, F), u32) for _ in range(2)]
          + [pltpu.VMEM((LA, SUB, D), f32) for _ in range(2)]
          + [pltpu.VMEM((SUB // 2, D), u32) for _ in range(6)]
          + [pltpu.VMEM((4, SUB, 128), f32) for _ in range(4)],
        compiler_params=pltpu.CompilerParams(vmem_limit_bytes=64 * 1024 * 1024),
    )(A_x.reshape(S, D), A_wqkv, A_wo, B_w1.T, B_b1, B_w2, B_b2)
    return out.reshape(1, S, D)
```

```python
import functools
import math

import jax
import jax.numpy as jnp
import jax.experimental.pallas as pl
import jax.experimental.pallas.tpu as pltpu

S, D, F = 2048, 512, 1376
H, DH, W, DIL = 32, 16, 8, 2
EPS = 1e-5
SCALE = DH ** -0.5
HALO = 16
SUB = 128
TM = 2 * SUB
NIT = S // TM
LA = 2
RB = 16
LB = 32
PR = 64
bf16, f32, u32, i32 = jnp.bfloat16, jnp.float32, jnp.uint32, jnp.int32


def _ln(x):
    m = jnp.sum(x, axis=-1, keepdims=True) * (1.0 / D)
    xc = x - m
    v = jnp.sum(xc * xc, axis=-1, keepdims=True) * (1.0 / D)
    return xc * jax.lax.rsqrt(v + EPS)


def _ln_ln(x):
    return _ln(_ln(x))


def _gelu(h):
    c = math.sqrt(2.0 / math.pi)
    u = h * (c + (c * 0.044715) * (h * h))
    hh = 0.5 * h
    return hh + hh * jnp.tanh(u)


def _tree(op, xs):
    xs = list(xs)
    while len(xs) > 1:
        nxt = [op(xs[k], xs[k + 1]) for k in range(0, len(xs) - 1, 2)]
        if len(xs) % 2:
            nxt.append(xs[-1])
        xs = nxt
    return xs[0]


def _recip(d):
    r = pl.reciprocal(d, approx=True)
    return r * (2.0 - d * r)


def _pk(v):
    return pltpu.bitcast(v.astype(bf16), u32)


def _up(v):
    return pltpu.bitcast(v, bf16)


def _sel4(sel, vals):
    return jnp.where(sel < 2, jnp.where(sel == 0, vals[0], vals[1]),
                     jnp.where(sel == 2, vals[2], vals[3]))


def _kernel(x_hbm, wqkv_hbm, wo_hbm, w1t_hbm, b1_hbm, w2_hbm, b2_hbm, o_hbm,
            x_v, o_v, wqkv_v, wo_v, w1t_v, w2_v, b1_v, b2_v,
            wqkv_p, wo_p, pt_s, zero_s, b1_s, b2_s, kv0_s, kv1_s, sem, osem, *bufs):
    x_s = bufs[0:2]
    g_s = bufs[2:4]
    x1_s = bufs[4:6]
    y2_s = bufs[6:8]
    y_s = bufs[8:12]
    q_s = bufs[12:16]

    def cp_x(lo, hi, s):
        return pltpu.make_async_copy(x_hbm.at[lo:hi], x_v.at[lo:hi], sem.at[s])

    cps = {
        'x0': cp_x(0, TM, 0),
        'Wq': pltpu.make_async_copy(wqkv_hbm.at[:, 0:D], wqkv_v.at[0], sem.at[1]),
        'Wk': pltpu.make_async_copy(wqkv_hbm.at[:, D:2 * D], wqkv_v.at[1], sem.at[2]),
        'Wv': pltpu.make_async_copy(wqkv_hbm.at[:, 2 * D:3 * D], wqkv_v.at[2], sem.at[3]),
        'wo': pltpu.make_async_copy(wo_hbm, wo_v, sem.at[4]),
        'x1': cp_x(TM, LA * TM, 5),
        'b1': pltpu.make_async_copy(b1_hbm, b1_v, sem.at[6]),
        'b2': pltpu.make_async_copy(b2_hbm, b2_v, sem.at[7]),
        'w1': pltpu.make_async_copy(w1t_hbm, w1t_v, sem.at[8]),
        'w2': pltpu.make_async_copy(w2_hbm, w2_v, sem.at[9]),
        'x2': cp_x(LA * TM, (LA + 1) * TM, 10),
    }
    cp_xr = cp_x((LA + 1) * TM, S, 11)

    def cp_out(row, n):
        return pltpu.make_async_copy(o_v.at[pl.ds(row, n)], o_hbm.at[pl.ds(row, n)], osem)

    for cp in cps.values():
        cp.start()

    kv0_s[:, 0:HALO, :] = jnp.zeros((8, HALO, 128), f32)
    kv1_s[:, 0:HALO, :] = jnp.zeros((8, HALO, 128), f32)
    zero_s[...] = jnp.zeros(zero_s.shape, i32)

    src_id = jax.lax.broadcasted_iota(i32, (128, 128), 1)
    dst_id = jax.lax.broadcasted_iota(i32, (128, 128), 0)
    for j in range(4):
        hit = dst_id == (src_id % 4) * 32 + (((src_id // 4) % 4 - j) % 4) * 8 + src_id // 16
        pt_s[j] = _pk(jnp.where(hit, 1.0, 0.0))

    def attn_block(ctx, rb, row0, tok, chain):
        b, kv, base = ctx
        r0 = rb * RB
        last = rb == SUB // RB - 1
        q = [q_s[b][c, r0:r0 + RB, :] for c in range(4)]
        lg = []
        for w in range(W):
            st = HALO + base + r0 - DIL * w
            s = _tree(jnp.add, [q[c] * kv[c, st:st + RB, :] for c in range(4)])
            s = s + pltpu.roll(s, 64, 1)
            s = s + pltpu.roll(s, 32, 1)
            if row0 is not None and r0 < DIL * w:
                pos = row0 + r0 + jax.lax.broadcasted_iota(i32, (RB, 128), 0)
                s = jnp.where(pos >= DIL * w, s, -1e9 / SCALE)
            lg.append(s)
        m = _tree(jnp.maximum, lg)
        e = [jnp.exp2((l - m) * (SCALE * math.log2(math.e))) for l in lg]
        inv = _recip(_tree(jnp.add, e))
        for c in range(4):
            st = HALO + base + r0
            acc = inv * _tree(jnp.add, [e[w] * kv[4 + c, st - DIL * w:st - DIL * w + RB, :]
                                        for w in range(W)])
            if chain and not last:
                tok = acc[0:8] if tok is None else tok + acc[0:8]
            elif chain and c == 3:
                acc = jnp.where(zero_s[...] == 0, acc, jnp.concatenate([tok] * (RB // 8), axis=0))
            y_s[b][r0 // 2:(r0 + RB) // 2, c * 128:(c + 1) * 128] = _pk(acc)
        return pltpu.roll(tok, 1, 1) if chain and not last else None

    def ln_stage(fn, load, ref):
        for r0 in range(0, SUB, LB):
            ref[r0 // 2:(r0 + LB) // 2, :] = _pk(fn(load(r0)))

    def rows(ref, *lead):
        return lambda r: ref[(*lead, slice(r, r + LB), slice(None))]

    def ln_in(b, row0):
        ln_stage(_ln, lambda r: x_v[pl.ds(row0 + r, LB), :].astype(f32), y_s[b])

    def st_q(ctx, lo=0, hi=3):
        b, kv, base = ctx
        qkv = jnp.dot(_up(y_s[b][...]), _up(wqkv_p[:, lo * D:hi * D]), preferred_element_type=f32)
        for c in range(4 * lo, 4 * hi):
            blk = qkv[:, c * 128 - lo * D:(c + 1) * 128 - lo * D]
            if c < 4:
                q_s[b][c] = blk
            else:
                kv[c - 4, HALO + base:HALO + base + SUB, :] = blk

    def attention(ctx, mask_row0, chain=True):
        tok = None
        for rb in range(SUB // RB):
            tok = attn_block(ctx, rb, mask_row0, tok, chain)

    def out_proj(ctx, lo=0, n=SUB):
        return jnp.dot(_up(y_s[ctx[0]][lo // 2:(lo + n) // 2, :]), _up(wo_p[...]),
                       preferred_element_type=f32)

    def halo(kv, n):
        kv[:, 0:HALO, :] = kv[:, n:n + HALO, :]

    def st_o1(ctx, j, row0, slot, mask_row0=None, parts=1):
        attention(ctx, mask_row0, chain=parts == 1)
        n = SUB // parts
        for lo in range(0, SUB, n):
            x1_s[j][slot, lo:lo + n, :] = (x_v[pl.ds(row0 + lo, n), :].astype(f32)
                                           + out_proj(ctx, lo, n))

    def ln2(j, slot):
        ln_stage(_ln_ln, rows(x1_s[j], slot), y2_s[j])

    def st_o2(ctx, j, mask_row0=None):
        attention(ctx, mask_row0)
        x_s[j][...] = x_s[j][...] + out_proj(ctx)
        ln_stage(_ln_ln, rows(x_s[j]), y_s[ctx[0]])

    def st_u(j, y):
        h = jax.lax.dot_general(_up(y), w1t_v[...], (((1,), (1,)), ((), ())),
                                preferred_element_type=f32) + b1_s[...]
        g_s[j][...] = _pk(_gelu(h))

    def mlp_out(j, lo=0, n=SUB):
        return jnp.dot(_up(g_s[j][lo // 2:(lo + n) // 2, :]), w2_v[...],
                       preferred_element_type=f32) + b2_s[...]

    def st_d1(j):
        x_s[j][...] = x1_s[j][0] + mlp_out(j)
        ln_stage(_ln, rows(x_s[j]), y_s[2 + j])
        x1_s[j][0] = x1_s[j][1]

    def st_d2(j, row0, parts=1):
        n = SUB // parts
        for lo in range(0, SUB, n):
            r = pl.multiple_of(row0 + lo, n)
            o_v[pl.ds(r, n), :] = (x_s[j][lo:lo + n, :] + mlp_out(j, lo, n)).astype(bf16)
            cp_out(r, n).start()

    ca = [(j, kv0_s, j * SUB) for j in range(2)]
    cm = [(2 + j, kv1_s, j * SUB) for j in range(2)]
    cb = [(2 + j, kv0_s, TM + j * SUB) for j in range(2)]

    def perm_cols(t):
        lane = jax.lax.broadcasted_iota(i32, (PR, 128), 1)
        for r in range(D // 2 // PR):
            src = [pltpu.bitcast(wqkv_v[t, 2 * r * PR:2 * (r + 1) * PR, c * 128:(c + 1) * 128], u32)
                   for c in range(4)]
            for j in range(4):
                mixed = _sel4(((lane // 4) % 4 - j) % 4, src)
                idx = (lane % 8) * 16 + (((lane // 8) + j) % 4) * 4 + lane // 32
                wqkv_p[r * PR:(r + 1) * PR, t * D + j * 128:t * D + (j + 1) * 128] = (
                    jnp.take_along_axis(mixed, idx, axis=1))

    def perm_wo():
        dhi = (jax.lax.broadcasted_iota(i32, (64, D), 0) // 2) % 4
        src = [pltpu.bitcast(wo_v[c * 128:(c + 1) * 128, :], u32) for c in range(4)]
        for j in range(4):
            mixed = _sel4((dhi - j) % 4, src)
            wo_p[j * 64:(j + 1) * 64, :] = _pk(
                jnp.dot(_up(pt_s[j]), _up(mixed), preferred_element_type=f32))

    ops = {
        'L0': lambda: (ln_in(0, 0), ln_in(1, SUB)),
        'L1': lambda: (ln_in(2, TM), ln_in(3, TM + SUB)),
        'W': perm_wo,
        'oX0': lambda: (st_o1(ca[0], 0, 0, 0, mask_row0=0), ln2(0, 0)),
        'oY0': lambda: st_o1(ca[1], 1, SUB, 0),
        'oX1': lambda: st_o1(cb[0], 0, TM, 1),
        'oY1': lambda: st_o1(cb[1], 1, TM + SUB, 1, parts=4),
    }
    for t, nm in enumerate('qkv'):
        ops['P' + nm] = functools.partial(perm_cols, t)
        for j, ch in enumerate('XY'):
            ops[nm + ch + '0'] = functools.partial(st_q, ca[j], t, t + 1)
            ops[nm + ch + '1'] = functools.partial(st_q, cb[j], t, t + 1)
    for name in ('!x0 L0 !Wq Pq qX0 !Wk Pk qY0 kX0 !Wv Pv kY0 vX0 !wo !x1 L1 vY0 W qX1 oX0 kX1 vX1 '
                 'oY0 qY1 kY1 vY1 oX1 oY1').split():
        if name[0] == '!':
            cps[name[1:]].wait()
        else:
            ops[name]()
    halo(kv0_s, LA * TM)
    cps['b1'].wait()
    cps['b2'].wait()
    b1_s[...] = b1_v[...].astype(f32).reshape(1, F)
    b2_s[...] = b2_v[...].astype(f32).reshape(1, D)
    cps['w1'].wait()
    cps['w2'].wait()
    cps['x2'].wait()
    cp_xr.start()

    def steady(k, ahead):
        rx = pl.multiple_of(k * TM, TM)
        ry = pl.multiple_of(rx + SUB, SUB)
        rn = pl.multiple_of(rx + LA * TM, TM)
        rm = pl.multiple_of(rn + SUB, SUB)
        st_u(0, y2_s[0][...])
        ln2(0, 1)
        if ahead:
            ln_in(0, rn)
            st_q(ca[0])
        st_d1(0)
        ln2(1, 0)
        st_u(1, y2_s[1][...])
        if ahead:
            st_o1(ca[0], 0, rn, 1)
        st_q(cm[0])
        st_d1(1)
        st_o2(cm[0], 0, mask_row0=rx if ahead else None)
        st_q(cm[1])
        st_u(0, y_s[2][...])
        st_o2(cm[1], 1)
        halo(kv1_s, TM)
        if ahead:
            ln_in(1, rm)
            st_q(ca[1])
        st_d2(0, rx)
        st_u(1, y_s[3][...])
        if ahead:
            st_o1(ca[1], 1, rm, 1)
            halo(kv0_s, TM)
        st_d2(1, ry, parts=1 if ahead else 2)

    def body1(k, carry):
        @pl.when(k == 1)
        def _():
            cp_xr.wait()
        steady(k, True)
        return carry

    def body2(k, carry):
        steady(k, False)
        return carry

    jax.lax.fori_loop(0, NIT - LA, body1, 0)
    jax.lax.fori_loop(NIT - LA, NIT, body2, 0)
    for k in range(NIT):
        cp_out(k * TM, SUB).wait()
        n = SUB if k < NIT - LA else SUB // 2
        for lo in range(0, SUB, n):
            cp_out(k * TM + SUB + lo, n).wait()


@jax.jit
def pallas_interleave_layers__sliding_local_dilated__mixer_channel_mlp__prompt_kernel(
    A_x: jax.Array,
    A_wqkv: jax.Array,
    A_wo: jax.Array,
    B_x: jax.Array,
    B_w1: jax.Array,
    B_b1: jax.Array,
    B_w2: jax.Array,
    B_b2: jax.Array,
):
    del B_x
    hbm = pl.BlockSpec(memory_space=pl.ANY)
    out = pl.pallas_call(
        _kernel,
        in_specs=[hbm] * 7,
        out_specs=hbm,
        out_shape=jax.ShapeDtypeStruct((S, D), bf16),
        scratch_shapes=[
            pltpu.VMEM((S, D), bf16),
            pltpu.VMEM((S, D), bf16),
            pltpu.VMEM((3, D, D), bf16),
            pltpu.VMEM((D, D), bf16),
            pltpu.VMEM((F, D), bf16),
            pltpu.VMEM((F, D), bf16),
            pltpu.VMEM((F,), bf16),
            pltpu.VMEM((D,), bf16),
            pltpu.VMEM((D // 2, 3 * D), u32),
            pltpu.VMEM((D // 2, D), u32),
            pltpu.VMEM((4, 64, 128), u32),
            pltpu.VMEM((RB, 128), i32),
            pltpu.VMEM((1, F), f32),
            pltpu.VMEM((1, D), f32),
            pltpu.VMEM((8, LA * TM + HALO, 128), f32),
            pltpu.VMEM((8, TM + HALO, 128), f32),
            pltpu.SemaphoreType.DMA((12,)),
            pltpu.SemaphoreType.DMA,
        ] + [pltpu.VMEM((SUB, D), f32) for _ in range(2)]
          + [pltpu.VMEM((SUB // 2, F), u32) for _ in range(2)]
          + [pltpu.VMEM((LA, SUB, D), f32) for _ in range(2)]
          + [pltpu.VMEM((SUB // 2, D), u32) for _ in range(6)]
          + [pltpu.VMEM((4, SUB, 128), f32) for _ in range(4)],
        compiler_params=pltpu.CompilerParams(vmem_limit_bytes=64 * 1024 * 1024),
    )(A_x.reshape(S, D), A_wqkv, A_wo, B_w1.T, B_b1, B_w2, B_b2)
    return out.reshape(1, S, D)
```
